```python
import os as _os
_os.environ.setdefault("JAX_PLATFORMS", "cpu")
import jax
import jax.numpy as jnp

def _softmax(x, axis=-1):
    return jax.nn.softmax(x, axis=axis)
def _gelu(x):
    return jax.nn.gelu(x, approximate=True)
def _silu(x):
    return jax.nn.silu(x)
def _sigmoid(x):
    return jax.nn.sigmoid(x)
def _layernorm(x, axis=-1, eps=1e-5):
    m = jnp.mean(x, axis=axis, keepdims=True)
    v = jnp.var(x, axis=axis, keepdims=True)
    return (x - m) / jnp.sqrt(v + eps)
def _scatter_add(tgt, idx, src, axis=0):
    return tgt.at[idx].add(src)
def _segment_sum(src, seg, n):
    return jax.ops.segment_sum(src, seg, n)
class _Rng:
    def __init__(self, key):
        self._k = key
    def _next(self):
        self._k, sub = jax.random.split(self._k)
        return sub
    def normal(self, shape):
        return jax.random.normal(self._next(), shape, dtype=jnp.bfloat16)
    def randint(self, lo, hi, shape):
        return jax.random.randint(self._next(), shape, lo, hi, dtype=jnp.int32)
    def uniform(self, shape, lo=0.0, hi=1.0):
        return jax.random.uniform(self._next(), shape, jnp.bfloat16, lo, hi)
    def permutation(self, n):
        return jax.random.permutation(self._next(), n)


kernel_name = 'recurrent_scan__ssm_conv_s4__mixer_s_mlp__prompt'

def setup_inputs():
    _rng = _Rng(jax.random.key(int.from_bytes(__import__("os").urandom(4), "little")))
    _w = (lambda a: (lambda t: t.astype(jnp.bfloat16) if jnp.issubdtype(t.dtype, jnp.floating) else t)(jnp.asarray(a)))
    def _A_setup():
        B, L, D, N = 1, 2048, 512, 128
        A_re = -jnp.exp((lambda *s: _rng.normal(s) * 0.1)(D, N))
        A_im = jnp.pi * (lambda *s: _rng.normal(s) * 0.1)(D, N)
        B_re = (lambda *s: _rng.normal(s) * 0.1)(D, N)
        B_im = (lambda *s: _rng.normal(s) * 0.1)(D, N)
        C_re = (lambda *s: _rng.normal(s) * 0.1)(D, N)
        C_im = (lambda *s: _rng.normal(s) * 0.1)(D, N)
        log_dt = (lambda *s: _rng.normal(s) * 0.1)(D) * 0.5 - 4.0
        Dskip = (lambda *s: _rng.normal(s) * 0.05)(D)
        return {
            "u": _w((lambda *s: _rng.normal(s) * 0.05)(B, L, D)),
            "A_re": _w(A_re),
            "A_im": _w(A_im),
            "B_re": _w(B_re),
            "B_im": _w(B_im),
            "C_re": _w(C_re),
            "C_im": _w(C_im),
            "log_dt": _w(log_dt),
            "Dskip": _w(Dskip),
        }
    _A_in = _A_setup()

    def _B_setup():
        B, S, D, F = 1, 2048, 512, 1376
        return {
            "x":  _w((lambda *s: _rng.normal(s) * 0.05)(B, S, D)),
            "w1": _w((lambda *s: _rng.normal(s) * 0.8)(D, D) * (D ** -0.5)),
            "w2": _w((lambda *s: _rng.normal(s) * 0.8)(D, D) * (D ** -0.5)),
            "w3": _w((lambda *s: _rng.normal(s) * 0.8)(D, F) * (D ** -0.5)),
            "w4": _w((lambda *s: _rng.normal(s) * 0.8)(F, D) * (F ** -0.5)),
        }
    _B_in = _B_setup()

    return {
        "A_u": _A_in["u"],
        "A_A_re": _A_in["A_re"],
        "A_A_im": _A_in["A_im"],
        "A_B_re": _A_in["B_re"],
        "A_B_im": _A_in["B_im"],
        "A_C_re": _A_in["C_re"],
        "A_C_im": _A_in["C_im"],
        "A_log_dt": _A_in["log_dt"],
        "A_Dskip": _A_in["Dskip"],
        "B_x": _B_in["x"],
        "B_w1": _B_in["w1"],
        "B_w2": _B_in["w2"],
        "B_w3": _B_in["w3"],
        "B_w4": _B_in["w4"],
    }

def reference(A_u, A_A_re, A_A_im, A_B_re, A_B_im, A_C_re, A_C_im, A_log_dt, A_Dskip, B_x, B_w1, B_w2, B_w3, B_w4):
    def _A_ref(u, A_re, A_im, B_re, B_im, C_re, C_im, log_dt, Dskip):
        Bsz, L, D = u.shape
        dt = jnp.exp(log_dt)[:, None]
        A = A_re + 1j * A_im
        Bc = B_re + 1j * B_im
        Cc = C_re + 1j * C_im
        logdA = dt * A
        dB = dt * Bc
        l = (lambda x, dt: x.astype(dt))(jnp.arange(L), A_re.dtype)
        P = jnp.exp(logdA[:, :, None] * l[None, None, :])
        K = jnp.einsum("dn,dnl,dn->dl", Cc, P, dB).real
        L2 = 2 * L
        Kp = jnp.pad(K, ((0, 0), (0, L)))
        up = (lambda x, *d: x.transpose(*d))(u, 0, 2, 1)
        up = jnp.pad(up, ((0, 0), (0, 0), (0, L)))
        Kf = (lambda x, axes=(-2,-1): jnp.fft.rfft2(x.astype(jnp.float32), axes=axes))(Kp[:, None, :], axes=(-2, -1))
        Uf = (lambda x, axes=(-2,-1): jnp.fft.rfft2(x.astype(jnp.float32), axes=axes))(up[:, :, None, :], axes=(-2, -1))
        Yf = Uf * Kf[None, :, :, :]
        y = (lambda x, s, axes=(-2,-1): jnp.fft.irfft2(x, s=s, axes=axes).astype(jnp.bfloat16))(Yf, (1, L2), axes=(-2, -1))[:, :, 0, :L]
        y = (lambda x, *d: x.transpose(*d))(y, 0, 2, 1) + u * Dskip[None, None, :]
        return y

    def _B_ref(x, w1, w2, w3, w4):
        B, S, D = x.shape
        h = _gelu(_layernorm(x, axis=-1) @ w1)
        c = D // 4
        g0 = jnp.pad(h[:, :, 0*c:1*c], ((0, 0), (1, 0), (0, 0)))[:, :S, :]
        g1 = jnp.pad(h[:, :, 1*c:2*c], ((0, 0), (0, 1), (0, 0)))[:, 1:, :]
        g2 = jnp.pad(h[:, :, 2*c:3*c], ((0, 0), (2, 0), (0, 0)))[:, :S, :]
        g3 = jnp.pad(h[:, :, 3*c:   ], ((0, 0), (0, 2), (0, 0)))[:, 2:, :]
        hs = jnp.concatenate([g0, g1, g2, g3], axis=-1) @ w2
        x1 = x + hs
        h2 = _gelu(_layernorm(x1, axis=-1) @ w3) @ w4
        return x1 + h2

    x = A_u
    xn = _layernorm(x, axis=-1)
    s = _A_ref(xn, A_A_re, A_A_im, A_B_re, A_B_im, A_C_re, A_C_im, A_log_dt, A_Dskip)
    g = _silu(_B_ref(xn, B_w1, B_w2, B_w3, B_w4))
    return x + s * g
```

```python
import functools

import numpy as np
import jax
import jax.numpy as jnp
import jax.experimental.pallas as pl
import jax.experimental.pallas.tpu as pltpu

F32 = jnp.float32
BF16 = jnp.bfloat16

L = 2048
D = 512
N = 128
FF = 1376
T = 128
NB = L // T
NH = 42
NLO = 16
NG = D // 8
RB = 256
HALO = 8


def _bf16_round(l):
    l = int(l)
    if l < 256:
        return l
    e = l.bit_length() - 8
    q, rem = l >> e, l & ((1 << e) - 1)
    half = 1 << (e - 1)
    if rem > half or (rem == half and (q & 1)):
        q += 1
    return q << e


def _hi_values():
    hi = []
    hi += [j for j in range(8)]
    hi += [128 + j for j in range(8)]
    hi += [256 + 128 * h + 2 * q for h in range(2) for q in range(4)]
    hi += [512 + 128 * h + 4 * q for h in range(4) for q in range(2)]
    hi += [1024 + 128 * h for h in range(8)]
    hi += [2048]
    return hi


@functools.lru_cache(maxsize=1)
def _tables():
    hi = _hi_values()
    pos = {}
    for h, hv in enumerate(hi):
        hb, j = h // 8, h % 8
        for lo in range(NLO):
            r = hv + 8 * lo
            lane = (8 * lo + 7 + j) % 128
            pos.setdefault(r, hb * 128 + lane)
    theta = np.pi * (2 * np.arange(T) + 1) / (2 * T)
    jj = np.arange(T)
    Fm = np.concatenate([np.cos(theta[:, None] * jj[None]), -np.sin(theta[:, None] * jj[None])], 0)
    mm = T + np.arange(T)
    Gm = np.concatenate([np.cos(mm[:, None] * theta[None]), -np.sin(mm[:, None] * theta[None])], 1) / T
    blocks, spans = [], []
    off = 0
    for b in range(NB):
        lags = [l for l in range((b - 1) * T + 1, (b + 1) * T) if 0 <= l < L]
        ps = [pos[_bf16_round(l)] for l in lags]
        t0, t1 = min(ps) // 128, max(ps) // 128
        nt = t1 - t0 + 1
        tab = np.zeros((2 * T, nt * 128), np.float64)
        for l, p in zip(lags, ps):
            m = l - (b - 1) * T
            tab[:T, p - t0 * 128] += np.cos(theta * m)
            tab[T:, p - t0 * 128] += -np.sin(theta * m)
        blocks.append(tab)
        spans.append((off, t0, nt))
        off += nt * 128
    Fx = np.concatenate(blocks, 1)
    return (Fm.astype(np.float32), Gm.astype(np.float32), Fx.astype(np.float32), tuple(spans))


def _cmul(ar, ai, br, bi):
    return ar * br - ai * bi, ar * bi + ai * br


def _ln(x):
    m = jnp.mean(x, axis=-1, keepdims=True)
    xc = x - m
    v = jnp.mean(xc * xc, axis=-1, keepdims=True)
    return xc * jax.lax.rsqrt(v + 1e-5)


def _gelu(x):
    return jax.nn.gelu(x, approximate=True)


def _make_kernel(spans, fx_cols):
    def kernel(are_ref, aim_ref, bre_ref, bim_ref, cre_ref, cim_ref, ldt_ref, dsk_ref,
               fm_ref, gm_ref,
               x_hbm, w1_hbm, w2_hbm, w3_hbm, w4_hbm, fx_hbm,
               out_hbm,
               x_v, w1_v, w2_v, w3_v, w4_v, fx_v, out_v,
               ehi_v, elo_v, kd_v, kdt_v, kh_v, uh_v, yh_v, xn_v, h_v,
               in_sems, out_sems):
        copies = [
            pltpu.make_async_copy(fx_hbm, fx_v, in_sems.at[0]),
            pltpu.make_async_copy(x_hbm, x_v, in_sems.at[1]),
            pltpu.make_async_copy(w1_hbm, w1_v, in_sems.at[2]),
            pltpu.make_async_copy(w2_hbm, w2_v, in_sems.at[3]),
            pltpu.make_async_copy(w3_hbm, w3_v, in_sems.at[4]),
            pltpu.make_async_copy(w4_hbm, w4_v, in_sems.at[5]),
        ]
        for c in copies:
            c.start()

        CB = 64
        rr = jax.lax.broadcasted_iota(jnp.int32, (CB, CB), 0)
        cc = jax.lax.broadcasted_iota(jnp.int32, (CB, CB), 1)
        prev = jnp.where(cc == (rr ^ 7), 1.0, 0.0).astype(BF16)

        def egen(cb, carry):
            r0 = pl.multiple_of(cb * CB, CB)
            g0 = pl.multiple_of(cb * (CB // 8), CB // 8)
            rows = pl.ds(r0, CB)
            ldt_b = ldt_ref[rows, :]
            are_b, aim_b = are_ref[rows, :], aim_ref[rows, :]

            def dtof(l):
                return jnp.exp(l.astype(F32)).astype(BF16).astype(F32)

            dt = dtof(ldt_b)
            ar = dt * are_b.astype(F32)
            ai = dt * aim_b.astype(F32)
            br = dt * bre_ref[rows, :].astype(F32)
            bi = dt * bim_ref[rows, :].astype(F32)
            cr, ci = _cmul(cre_ref[rows, :].astype(F32), cim_ref[rows, :].astype(F32), br, bi)

            def zpow(ar_, ai_, k):
                mag = jnp.exp(ar_ * k)
                return mag * jnp.cos(ai_ * k), mag * jnp.sin(ai_ * k)

            z1 = zpow(ar, ai, 1.0)
            v = zpow(ar, ai, 128.0)
            pw = [None, z1]
            for j in range(2, 8):
                pw.append(_cmul(*pw[-1], *z1))

            def put_hi(h, val):
                ehi_v[pl.ds(g0, CB // 8), h, :, 0:N] = val[0].reshape(CB // 8, 8, N)
                ehi_v[pl.ds(g0, CB // 8), h, :, N:2 * N] = val[1].reshape(CB // 8, 8, N)

            cv = (cr, ci)
            for hp in range(17):
                if hp < 2:
                    js, h0 = list(range(8)), 8 * hp
                elif hp < 4:
                    js, h0 = [0, 2, 4, 6], 16 + 4 * (hp - 2)
                elif hp < 8:
                    js, h0 = [0, 4], 24 + 2 * (hp - 4)
                else:
                    js, h0 = [0], 32 + (hp - 8)
                for q, j in enumerate(js):
                    put_hi(h0 + q, cv if j == 0 else _cmul(*cv, *pw[j]))
                if hp < 16:
                    cv = _cmul(*cv, *v)
            zero = jnp.zeros((CB, N), F32)
            put_hi(NH - 1, (zero, zero))

            def rev(a):
                return jnp.dot(prev, a, preferred_element_type=F32)

            dtr = dtof(rev(ldt_b))
            arr = dtr * rev(are_b)
            air = dtr * rev(aim_b)
            w = zpow(arr, air, 8.0)
            wp = (jnp.ones((CB, N), F32), zero)
            for lo in range(NLO):
                elo_v[pl.ds(g0, CB // 8), lo, :, 0:N] = wp[0].reshape(CB // 8, 8, N)
                elo_v[pl.ds(g0, CB // 8), lo, :, N:2 * N] = (-wp[1]).reshape(CB // 8, 8, N)
                if lo == 0:
                    wp = w
                elif lo < NLO - 1:
                    wp = _cmul(*wp, *w)
            return carry

        jax.lax.fori_loop(0, D // CB, egen, 0)

        lane8 = jax.lax.broadcasted_iota(jnp.int32, (8, 128), 1) % 8

        def kgen(g, carry):
            lhs = ehi_v[g].reshape(NH * 8, 2 * N).astype(BF16)
            rhs = elo_v[g].reshape(NLO * 8, 2 * N).astype(BF16)
            o = jax.lax.dot_general(lhs, rhs, (((1,), (1,)), ((), ())), preferred_element_type=F32)
            r0 = pl.multiple_of(g * 8, 8)
            for hb in range(6):
                acc = jnp.zeros((8, 128), F32)
                for j in range(8):
                    h = 8 * hb + j
                    if h >= NH - 1:
                        continue
                    blk = pltpu.roll(o[8 * h:8 * h + 8, :], j, 1, stride=1, stride_axis=0)
                    acc = jnp.where(lane8 == (7 + j) % 8, blk, acc)
                kd_v[pl.ds(r0, 8), hb * 128:(hb + 1) * 128] = acc
            return carry

        jax.lax.fori_loop(0, NG, kgen, 0)
        kdt_v[...] = kd_v[...].T.astype(BF16)

        copies[0].wait()
        for b, (off, t0, nt) in enumerate(spans):
            kh_v[b] = jnp.dot(fx_v[:, off:off + nt * 128], kdt_v[t0 * 128:(t0 + nt) * 128, :],
                              preferred_element_type=F32)

        copies[1].wait()
        copies[2].wait()
        h_v[0:HALO, :] = jnp.zeros((HALO, D), F32)
        h_v[HALO + L:HALO + L + HALO, :] = jnp.zeros((HALO, D), F32)

        def p1a(k, carry):
            r0 = pl.multiple_of(k * RB, RB)
            xn = _ln(x_v[pl.ds(r0, RB), :].astype(F32)).astype(BF16)
            xn_v[pl.ds(r0, RB), :] = xn
            xn2 = _ln(xn.astype(F32)).astype(BF16)
            h = _gelu(jnp.dot(xn2, w1_v[...], preferred_element_type=F32))
            h_v[pl.ds(pl.multiple_of(r0 + HALO, 8), RB), :] = h
            for c in range(RB // T):
                uh_v[k * (RB // T) + c] = jnp.dot(fm_ref[...], xn[c * T:(c + 1) * T, :],
                                                  preferred_element_type=F32)
            return carry

        jax.lax.fori_loop(0, L // RB, p1a, 0)

        copies[3].wait()
        copies[4].wait()
        copies[5].wait()
        C4 = D // 4
        R = 8

        def p1b(k, carry):
            lo_c = k
            hi_c = NB - 1 - k
            for sb in range(0, T, R):
                re_s, im_s = pl.ds(sb, R), pl.ds(T + sb, R)

                def prod(b, i):
                    kr, ki = kh_v[b, re_s, :], kh_v[b, im_s, :]
                    ur, ui = uh_v[i, re_s, :], uh_v[i, im_s, :]
                    return kr * ur - ki * ui, kr * ui + ki * ur

                alr, ali = prod(0, lo_c)
                ahr, ahi = prod(0, hi_c)
                for b in range(1, 9):
                    pr, pi_ = prod(b, hi_c - b)
                    ahr, ahi = ahr + pr, ahi + pi_
                for s in range(1, 8):
                    is_lo = s <= k
                    b = jnp.where(is_lo, s, s - k + 8)
                    i = jnp.where(is_lo, k - s, NB - 1 - k - (s - k + 8))
                    pr, pi_ = prod(b, i)
                    m = jnp.where(is_lo, 1.0, 0.0).astype(F32)
                    alr, ali = alr + m * pr, ali + m * pi_
                    ahr, ahi = ahr + (1.0 - m) * pr, ahi + (1.0 - m) * pi_
                yh_v[0, re_s, :] = alr
                yh_v[0, im_s, :] = ali
                yh_v[1, re_s, :] = ahr
                yh_v[1, im_s, :] = ahi

            rows = [pl.multiple_of(lo_c * T, T), pl.multiple_of(hi_c * T, T)]
            ys, xns, xs, hss = [], [], [], []
            for c in range(2):
                ys.append(jnp.dot(gm_ref[...], yh_v[c].astype(BF16), preferred_element_type=F32))
                xns.append(xn_v[pl.ds(rows[c], T), :])
                xs.append(x_v[pl.ds(rows[c], T), :])
                win = h_v[pl.ds(rows[c], T + 2 * HALO), :]
                hss.append(jnp.concatenate([
                    win[HALO - 1:HALO - 1 + T, 0 * C4:1 * C4],
                    win[HALO + 1:HALO + 1 + T, 1 * C4:2 * C4],
                    win[HALO - 2:HALO - 2 + T, 2 * C4:3 * C4],
                    win[HALO + 2:HALO + 2 + T, 3 * C4:4 * C4]], axis=-1).astype(BF16))
            y = jnp.concatenate(ys, 0).astype(BF16)
            xn = jnp.concatenate(xns, 0)
            x = jnp.concatenate(xs, 0)
            hs = jnp.concatenate(hss, 0)
            xnf = xn.astype(F32)
            s = y.astype(F32) + xnf * dsk_ref[...].astype(F32)
            x1 = xnf + jnp.dot(hs, w2_v[...], preferred_element_type=F32)
            h3 = _gelu(jnp.dot(_ln(x1).astype(BF16), w3_v[...], preferred_element_type=F32))
            bb = x1 + jnp.dot(h3.astype(BF16), w4_v[...], preferred_element_type=F32)
            o = (x.astype(F32) + s * (bb * jax.nn.sigmoid(bb))).astype(BF16)
            for c, ci in enumerate((lo_c, hi_c)):
                out_v[pl.ds(rows[c], T), :] = o[c * T:(c + 1) * T, :]
                pltpu.make_async_copy(out_v.at[pl.ds(rows[c], T), :], out_hbm.at[pl.ds(rows[c], T), :],
                                      out_sems.at[ci]).start()
            return carry

        jax.lax.fori_loop(0, NB // 2, p1b, 0)

        for ci in range(NB):
            pltpu.make_async_copy(out_v.at[pl.ds(ci * T, T), :], out_hbm.at[pl.ds(ci * T, T), :],
                                  out_sems.at[ci]).wait()

    return kernel


@jax.jit
def pallas_recurrent_scan__ssm_conv_s4__mixer_s_mlp__prompt_kernel(
    A_u: jax.Array,
    A_A_re: jax.Array,
    A_A_im: jax.Array,
    A_B_re: jax.Array,
    A_B_im: jax.Array,
    A_C_re: jax.Array,
    A_C_im: jax.Array,
    A_log_dt: jax.Array,
    A_Dskip: jax.Array,
    B_x: jax.Array,
    B_w1: jax.Array,
    B_w2: jax.Array,
    B_w3: jax.Array,
    B_w4: jax.Array,
):
    Fm, Gm, Fx, spans = _tables()
    fx_cols = Fx.shape[1]
    x = A_u.reshape(L, D)
    ldt = jnp.broadcast_to(A_log_dt.reshape(D, 1), (D, N))
    dsk = A_Dskip.reshape(1, D)

    vm = pl.BlockSpec(memory_space=pltpu.VMEM)
    hbm = pl.BlockSpec(memory_space=pl.ANY)
    out = pl.pallas_call(
        _make_kernel(spans, fx_cols),
        out_shape=jax.ShapeDtypeStruct((L, D), BF16),
        in_specs=[vm] * 10 + [hbm] * 6,
        out_specs=hbm,
        scratch_shapes=[
            pltpu.VMEM((L, D), BF16),
            pltpu.VMEM((D, D), BF16),
            pltpu.VMEM((D, D), BF16),
            pltpu.VMEM((D, FF), BF16),
            pltpu.VMEM((FF, D), BF16),
            pltpu.VMEM((2 * T, fx_cols), BF16),
            pltpu.VMEM((L, D), BF16),
            pltpu.VMEM((NG, NH, 8, 2 * N), F32),
            pltpu.VMEM((NG, NLO, 8, 2 * N), F32),
            pltpu.VMEM((D, 6 * 128), F32),
            pltpu.VMEM((6 * 128, D), BF16),
            pltpu.VMEM((NB, 2 * T, D), F32),
            pltpu.VMEM((NB, 2 * T, D), F32),
            pltpu.VMEM((2, 2 * T, D), F32),
            pltpu.VMEM((L, D), BF16),
            pltpu.VMEM((L + 2 * HALO, D), F32),
            pltpu.SemaphoreType.DMA((6,)),
            pltpu.SemaphoreType.DMA((NB,)),
        ],
        compiler_params=pltpu.CompilerParams(vmem_limit_bytes=100 * 1024 * 1024),
    )(A_A_re, A_A_im, A_B_re, A_B_im, A_C_re, A_C_im, ldt, dsk,
      jnp.asarray(Fm, BF16), jnp.asarray(Gm, BF16),
      x, B_w1, B_w2, B_w3, B_w4, jnp.asarray(Fx, BF16))
    return out.reshape(1, L, D)
```

```python
import functools

import numpy as np
import jax
import jax.numpy as jnp
import jax.experimental.pallas as pl
import jax.experimental.pallas.tpu as pltpu

F32 = jnp.float32


def _mo(x, m):
    return x if isinstance(x, int) else pl.multiple_of(x, m)


BF16 = jnp.bfloat16

L = 2048
D = 512
N = 128
FF = 1376
T = 128
NB = L // T
NH = 42
NLO = 16
NG = D // 8
RB = 256
HALO = 8


def _bf16_round(l):
    l = int(l)
    if l < 256:
        return l
    e = l.bit_length() - 8
    q, rem = l >> e, l & ((1 << e) - 1)
    half = 1 << (e - 1)
    if rem > half or (rem == half and (q & 1)):
        q += 1
    return q << e


def _hi_values():
    hi = []
    hi += [j for j in range(8)]
    hi += [128 + j for j in range(8)]
    hi += [256 + 128 * h + 2 * q for h in range(2) for q in range(4)]
    hi += [512 + 128 * h + 4 * q for h in range(4) for q in range(2)]
    hi += [1024 + 128 * h for h in range(8)]
    hi += [2048]
    return hi


@functools.lru_cache(maxsize=1)
def _tables():
    hi = _hi_values()
    pos = {}
    for h, hv in enumerate(hi):
        hb, j = h // 8, h % 8
        for lo in range(NLO):
            r = hv + 8 * lo
            lane = 8 * lo + j
            pos.setdefault(r, hb * 128 + lane)
    theta = np.pi * (2 * np.arange(T) + 1) / (2 * T)
    jj = np.arange(T)
    Fm = np.concatenate([np.cos(theta[:, None] * jj[None]), -np.sin(theta[:, None] * jj[None])], 0)
    mm = T + np.arange(T)
    Gm = np.concatenate([np.cos(mm[:, None] * theta[None]), -np.sin(mm[:, None] * theta[None])], 1) / T
    blocks, spans = [], []
    off = 0
    for b in range(NB):
        lags = [l for l in range((b - 1) * T + 1, (b + 1) * T) if 0 <= l < L]
        ps = [pos[_bf16_round(l)] for l in lags]
        t0, t1 = min(ps) // 128, max(ps) // 128
        nt = t1 - t0 + 1
        tab = np.zeros((2 * T, nt * 128), np.float64)
        for l, p in zip(lags, ps):
            m = l - (b - 1) * T
            tab[:T, p - t0 * 128] += np.cos(theta * m)
            tab[T:, p - t0 * 128] += -np.sin(theta * m)
        blocks.append(tab)
        spans.append((off, t0, nt))
        off += nt * 128
    Fx = np.concatenate(blocks, 1)
    return (Fm.astype(np.float32), Gm.astype(np.float32), Fx.astype(np.float32), tuple(spans))


def _cmul(ar, ai, br, bi):
    return ar * br - ai * bi, ar * bi + ai * br


def _sincos(x):
    kf = jnp.floor(x * 0.6366197723675814 + 0.5)
    r = x - kf * 1.5703125
    r = r - kf * 4.837512969970703125e-4
    r = r - kf * 7.54978995489188216e-8
    r2 = r * r
    s = r + r * r2 * (-1.6666654611e-1 + r2 * (8.3321608736e-3 + r2 * (-1.9515295891e-4)))
    c = 1.0 - 0.5 * r2 + r2 * r2 * (4.166664568298827e-2 + r2 * (-1.388731625493765e-3 + r2 * 2.443315711809948e-5))
    q = kf.astype(jnp.int32)
    swap = (q & 1) == 1
    sn = jnp.where(swap, c, s)
    cs = jnp.where(swap, s, c)
    sn = jnp.where((q & 2) == 2, -sn, sn)
    cs = jnp.where(((q + 1) & 2) == 2, -cs, cs)
    return sn, cs


def _ln(x):
    m = jnp.mean(x, axis=-1, keepdims=True)
    xc = x - m
    v = jnp.mean(xc * xc, axis=-1, keepdims=True)
    return xc * jax.lax.rsqrt(v + 1e-5)


def _gelu(x):
    c1 = 0.7978845608028654
    u = x * (x * x * (c1 * 0.044715) + c1)
    hx = 0.5 * x
    return hx + hx * jnp.tanh(u)


def _make_kernel(spans, fx_cols):
    def kernel(are_ref, aim_ref, bre_ref, bim_ref, cre_ref, cim_ref, ldt_ref, dsk_ref,
               fm_ref, gm_ref,
               x_hbm, w1_hbm, w2_hbm, w3_hbm, w4_hbm, fx_hbm,
               out_hbm,
               x_v, w1_v, w2_v, w3_v, w4_v, fx_v, out_v,
               ehi_v, elo_v, kd_v, kdt_v, kh_v, uh_v, yh_v, xn_v, h_v,
               ldt_v, acc_v, x1n_v, kd2_v, in_sems, out_sems):
        def xcopy(k):
            r = pl.ds(_mo(k * RB, RB), RB)
            return pltpu.make_async_copy(x_hbm.at[r, :], x_v.at[r, :], in_sems.at[5 + k])

        copies = [
            pltpu.make_async_copy(fx_hbm, fx_v, in_sems.at[0]),
            pltpu.make_async_copy(w1_hbm, w1_v, in_sems.at[1]),
            pltpu.make_async_copy(w2_hbm, w2_v, in_sems.at[2]),
            pltpu.make_async_copy(w3_hbm, w3_v, in_sems.at[3]),
            pltpu.make_async_copy(w4_hbm, w4_v, in_sems.at[4]),
        ]
        xcopy(0).start()
        copies[1].start()
        for k in range(1, L // RB):
            xcopy(k).start()
        for c in (0, 2, 3, 4):
            copies[c].start()

        ld_row = ldt_ref[...].astype(F32).reshape(1, D)
        ldt_v[...] = jnp.broadcast_to(ld_row, (N, D)).T.astype(BF16)

        CB = 64

        def egen(cb, carry):
            r0 = _mo(cb * CB, CB)
            rows = pl.ds(r0, CB)
            ldt_b = ldt_v[rows, :]
            are_b, aim_b = are_ref[rows, :], aim_ref[rows, :]

            def dtof(l):
                return jnp.exp(l.astype(F32)).astype(BF16).astype(F32)

            def zpow(ar_, ai_, k):
                mag = jnp.exp(ar_ * k)
                sn, cs = _sincos(ai_ * k)
                return mag * cs, mag * sn

            dt_a = dtof(ldt_b)
            for gg in range(CB // 8):
                g = cb * (CB // 8) + gg
                sl = slice(8 * gg, 8 * gg + 8)
                rg = pl.ds(_mo(r0 + 8 * gg, 8), 8)
                dt = dt_a[sl]
                ar = dt * are_b[sl].astype(F32)
                ai = dt * aim_b[sl].astype(F32)
                br = dt * bre_ref[rg, :].astype(F32)
                bi = dt * bim_ref[rg, :].astype(F32)
                cr, ci = _cmul(cre_ref[rg, :].astype(F32), cim_ref[rg, :].astype(F32), br, bi)
                z1 = zpow(ar, ai, 1.0)
                pw = [None, z1]
                for j in range(2, 8):
                    pw.append(_cmul(*pw[-1], *z1))
                w = (pw[4][0] * pw[4][0] - pw[4][1] * pw[4][1], 2.0 * pw[4][0] * pw[4][1])
                v = w
                for _ in range(4):
                    v = (v[0] * v[0] - v[1] * v[1], 2.0 * v[0] * v[1])
                pend = []

                def pack2(ref, idx, v0, v1):
                    for p, ls in ((0, slice(0, N)), (1, slice(N, 2 * N))):
                        ref[g, idx, :, ls] = jnp.concatenate([v0[p], v1[p]], axis=0).astype(BF16)

                def put_hi(h, val):
                    pend.append(val)
                    if h % 2 == 1:
                        pack2(ehi_v, h // 2, pend[0], pend[1])
                        pend.clear()

                cv = (cr, ci)
                for hp in range(17):
                    if hp < 2:
                        js, h0 = list(range(8)), 8 * hp
                    elif hp < 4:
                        js, h0 = [0, 2, 4, 6], 16 + 4 * (hp - 2)
                    elif hp < 8:
                        js, h0 = [0, 4], 24 + 2 * (hp - 4)
                    else:
                        js, h0 = [0], 32 + (hp - 8)
                    for q, j in enumerate(js):
                        put_hi(h0 + q, cv if j == 0 else _cmul(*cv, *pw[j]))
                    if hp < 16:
                        cv = _cmul(*cv, *v)
                zero = jnp.zeros((8, N), F32)
                put_hi(NH - 1, (zero, zero))

                wp = (jnp.ones((8, N), F32), zero)
                prevv = None
                for lo in range(NLO):
                    cur = (wp[0], -wp[1])
                    if lo % 2 == 1:
                        pack2(elo_v, lo // 2, prevv, cur)
                    prevv = cur
                    if lo == 0:
                        wp = w
                    elif lo < NLO - 1:
                        wp = _cmul(*wp, *w)
            return carry

        lane8 = jax.lax.broadcasted_iota(jnp.int32, (8, 128), 1) % 8

        KG = 8

        def kgen(gi, carry):
            for gg in range(KG):
                g = gi * KG + gg
                lhs = ehi_v[g].reshape(NH * 8, 2 * N)
                rhs = elo_v[g].reshape(NLO * 8, 2 * N)
                o = jax.lax.dot_general(lhs, rhs, (((1,), (1,)), ((), ())), preferred_element_type=F32)
                r0 = _mo(g * 8, 8)
                for hb in range(6):
                    acc = jnp.zeros((8, 128), F32)
                    for j in range(8):
                        h = 8 * hb + j
                        if h >= NH - 1:
                            continue
                        blk = pltpu.roll(o[8 * h:8 * h + 8, :], j, 1, stride=7, stride_axis=0)
                        acc = jnp.where(lane8 == j, blk, acc)
                    kd_v[pl.ds(r0, 8), hb * 128:(hb + 1) * 128] = acc
            return carry


        h_v[0:HALO, :] = jnp.zeros((HALO, D), F32)
        for p in range(3):
            uh_v[NB, p] = jnp.zeros((T, D), F32)
        h_v[HALO + L:HALO + L + HALO, :] = jnp.zeros((HALO, D), F32)

        def p1a(k, carry):
            r0 = _mo(k * RB, RB)
            xn = _ln(x_v[pl.ds(r0, RB), :].astype(F32)).astype(BF16)
            xn_v[pl.ds(r0, RB), :] = xn
            xn2 = _ln(xn.astype(F32)).astype(BF16)
            h = _gelu(jnp.dot(xn2, w1_v[...], preferred_element_type=F32))
            h_v[pl.ds(_mo(r0 + HALO, 8), RB), :] = h
            for c in range(RB // T):
                uu = jnp.dot(fm_ref[...], xn[c * T:(c + 1) * T, :], preferred_element_type=F32)
                ci = k * (RB // T) + c
                uh_v[ci, 0] = uu[:T] + uu[T:]
                uh_v[ci, 1] = uu[:T]
                uh_v[ci, 2] = uu[T:]
            return carry

        egen(0, 0)
        egen(1, 0)
        kgen(0, 0)
        copies[1].wait()

        def merged(k, carry):
            xcopy(k - 1).wait()
            egen(k + 1, 0)
            kgen(k, 0)
            p1a(k - 1, 0)
            return carry

        jax.lax.fori_loop(1, L // RB - 1, merged, 0)
        xcopy(L // RB - 2).wait()
        xcopy(L // RB - 1).wait()
        kgen(L // RB - 1, 0)
        p1a(L // RB - 2, 0)
        p1a(L // RB - 1, 0)
        lane8w = jax.lax.broadcasted_iota(jnp.int32, (8, D), 1) % 8
        for tl in range(6):
            kt = kd_v[:, tl * 128:(tl + 1) * 128].T
            for i in range(16):
                o_ = kt[8 * i:8 * i + 8, :]
                for r in range(1, 8):
                    i2 = (i + r) % 16
                    o_ = jnp.where(lane8w == r, kt[8 * i2:8 * i2 + 8, :], o_)
                kd2_v[tl * 128 + 8 * i:tl * 128 + 8 * i + 8, :] = o_
        kdt_v[...] = kd2_v[...].astype(BF16)

        copies[0].wait()
        for b, (off, t0, nt) in enumerate(spans):
            kk = jnp.dot(fx_v[:, off:off + nt * 128], kdt_v[t0 * 128:(t0 + nt) * 128, :],
                         preferred_element_type=F32)
            kc, kd_ = kk[:T], kk[T:]
            kh_v[b, 0] = kc
            kh_v[b, 1] = kd_ - kc
            kh_v[b, 2] = kc + kd_


        copies[2].wait()
        copies[3].wait()
        copies[4].wait()
        C4 = D // 4
        R = 8

        LH = 256

        def p1b(m, carry):
            rows = [_mo(m * RB, RB), _mo((NB // 2 - 1 - m) * RB, RB)]
            split = 2 * m + 2

            def pointwise(sbi):
                if isinstance(sbi, int):
                    sb, l0 = (sbi // 2) * R, (sbi % 2) * LH
                else:
                    sb, l0 = _mo((sbi // 2) * R, R), _mo((sbi % 2) * LH, LH)
                rs = pl.ds(sb, R)
                rs2 = pl.ds(_mo(sb + T, R), R)
                ls = pl.ds(l0, LH)

                def ldu(i):
                    return [uh_v[i, p, rs, ls] for p in range(3)]

                accA = accB = snap = None
                ucur = None
                for s in range(NB + 2):
                    if s < 2:
                        b, top = s, 2 * m + 1
                    elif s >= 8:
                        b, top = s - split, NB - 1 - 2 * m
                    else:
                        first = s < split
                        b = jnp.where(first, s, s - split)
                        top = jnp.where(first, 2 * m + 1, NB - 1 - 2 * m)
                    if s in (2, 4, 6, 8):
                        if snap is None:
                            snap = accA + accB
                        else:
                            at = split == s
                            snap = [jnp.where(at, x_, y_) for x_, y_ in zip(accA + accB, snap)]
                    if s in (0, 2, 4, 6, 8):
                        ucur = ldu(top - b)
                    kk = [kh_v[b, p, rs, ls] for p in range(3)]
                    pa = [k_ * u_ for k_, u_ in zip(kk, ucur)]
                    accA = pa if accA is None else [x_ + y_ for x_, y_ in zip(accA, pa)]
                    if s == NB + 1:
                        break
                    nxt = top - b - 1
                    if s <= 7:
                        nxt = jnp.where(nxt < 0, NB, nxt)
                    unext = ldu(nxt)
                    pb = [k_ * u_ for k_, u_ in zip(kk, unext)]
                    accB = pb if accB is None else [x_ + y_ for x_, y_ in zip(accB, pb)]
                    ucur = unext
                tot = accA + accB
                sec = [x_ - y_ for x_, y_ in zip(tot, snap)]
                for c, ss in ((1, snap[0:3]), (0, snap[3:6]), (3, sec[0:3]), (2, sec[3:6])):
                    yh_v[c, rs, ls] = ss[0] - ss[2]
                    yh_v[c, rs2, ls] = ss[0] + ss[1]

            xns, hss = [], []
            for c in range(2):
                xns.append(xn_v[pl.ds(rows[c], RB), :])
                win = h_v[pl.ds(rows[c], RB + 2 * HALO), :]
                hss.append(jnp.concatenate([
                    win[HALO - 1:HALO - 1 + RB, 0 * C4:1 * C4],
                    win[HALO + 1:HALO + 1 + RB, 1 * C4:2 * C4],
                    win[HALO - 2:HALO - 2 + RB, 2 * C4:3 * C4],
                    win[HALO + 2:HALO + 2 + RB, 3 * C4:4 * C4]], axis=-1).astype(BF16))
            hs = jnp.concatenate(hss, 0)
            x1 = jnp.concatenate(xns, 0).astype(F32) + jnp.dot(hs, w2_v[...], preferred_element_type=F32)
            acc_v[...] = x1
            x1n_v[...] = _ln(x1).astype(BF16)
            FC, PRE, INN = 384, 6, 8
            for q in range(PRE):
                pointwise(q)

            def ffchunk(w3c, w4c):
                h3 = _gelu(jax.lax.dot_general(x1n_v[...], w3c, (((1,), (1,)), ((), ())),
                                               preferred_element_type=F32))
                acc_v[...] += jnp.dot(h3.astype(BF16), w4c, preferred_element_type=F32)

            def inner(c, carry2):
                c0 = _mo(c * FC, 16)
                ffchunk(w3_v[pl.ds(c0, FC), :], w4_v[pl.ds(c0, FC), :])
                for q in range(INN):
                    pointwise(PRE + INN * c + q)
                return carry2

            NFC = FF // FC
            jax.lax.fori_loop(0, NFC, inner, 0)
            if NFC * FC < FF:
                ffchunk(w3_v[NFC * FC:FF, :], w4_v[NFC * FC:FF, :])
            for q in range(PRE + INN * NFC, 2 * T // R):
                pointwise(q)
            for c in range(2):
                ys = [jnp.dot(gm_ref[...], yh_v[2 * c + q].astype(BF16), preferred_element_type=F32)
                      for q in range(2)]
                y = jnp.concatenate(ys, 0).astype(BF16)
                bb = acc_v[c * RB:(c + 1) * RB, :]
                xnf = xn_v[pl.ds(rows[c], RB), :].astype(F32)
                s = y.astype(F32) + xnf * dsk_ref[...].astype(F32).reshape(1, D)
                o = x_v[pl.ds(rows[c], RB), :].astype(F32) + s * (bb * jax.nn.sigmoid(bb))
                out_v[pl.ds(rows[c], RB), :] = o.astype(BF16)
                ci = m if c == 0 else NB // 2 - 1 - m
                pltpu.make_async_copy(out_v.at[pl.ds(rows[c], RB), :], out_hbm.at[pl.ds(rows[c], RB), :],
                                      out_sems.at[ci]).start()
            return carry

        jax.lax.fori_loop(0, NB // 4, p1b, 0)

        for ci in range(NB // 2):
            pltpu.make_async_copy(out_v.at[pl.ds(ci * RB, RB), :], out_hbm.at[pl.ds(ci * RB, RB), :],
                                  out_sems.at[ci]).wait()

    return kernel


@jax.jit
def pallas_recurrent_scan__ssm_conv_s4__mixer_s_mlp__prompt_kernel(
    A_u: jax.Array,
    A_A_re: jax.Array,
    A_A_im: jax.Array,
    A_B_re: jax.Array,
    A_B_im: jax.Array,
    A_C_re: jax.Array,
    A_C_im: jax.Array,
    A_log_dt: jax.Array,
    A_Dskip: jax.Array,
    B_x: jax.Array,
    B_w1: jax.Array,
    B_w2: jax.Array,
    B_w3: jax.Array,
    B_w4: jax.Array,
):
    Fm, Gm, Fx, spans = _tables()
    fx_cols = Fx.shape[1]
    x = A_u.reshape(L, D)

    vm = pl.BlockSpec(memory_space=pltpu.VMEM)
    hbm = pl.BlockSpec(memory_space=pl.ANY)
    out = pl.pallas_call(
        _make_kernel(spans, fx_cols),
        out_shape=jax.ShapeDtypeStruct((L, D), BF16),
        in_specs=[vm] * 10 + [hbm] * 6,
        out_specs=hbm,
        scratch_shapes=[
            pltpu.VMEM((L, D), BF16),
            pltpu.VMEM((D, D), BF16),
            pltpu.VMEM((D, D), BF16),
            pltpu.VMEM((FF, D), BF16),
            pltpu.VMEM((FF, D), BF16),
            pltpu.VMEM((2 * T, fx_cols), BF16),
            pltpu.VMEM((L, D), BF16),
            pltpu.VMEM((NG, NH // 2, 16, 2 * N), BF16),
            pltpu.VMEM((NG, NLO // 2, 16, 2 * N), BF16),
            pltpu.VMEM((D, 6 * 128), F32),
            pltpu.VMEM((6 * 128, D), BF16),
            pltpu.VMEM((NB, 3, T, D), F32),
            pltpu.VMEM((NB + 1, 3, T, D), F32),
            pltpu.VMEM((4, 2 * T, D), F32),
            pltpu.VMEM((L, D), BF16),
            pltpu.VMEM((L + 2 * HALO, D), F32),
            pltpu.VMEM((D, N), BF16),
            pltpu.VMEM((2 * RB, D), F32),
            pltpu.VMEM((2 * RB, D), BF16),
            pltpu.VMEM((6 * 128, D), F32),
            pltpu.SemaphoreType.DMA((5 + L // RB,)),
            pltpu.SemaphoreType.DMA((NB // 2,)),
        ],
        compiler_params=pltpu.CompilerParams(vmem_limit_bytes=100 * 1024 * 1024),
    )(A_A_re, A_A_im, A_B_re, A_B_im, A_C_re, A_C_im, A_log_dt, A_Dskip,
      jnp.asarray(Fm, BF16), jnp.asarray(Gm, BF16),
      x, B_w1, B_w2, B_w3.T, B_w4, jnp.asarray(Fx, BF16))
    return out.reshape(1, L, D)
```

```python
import functools

import numpy as np
import jax
import jax.numpy as jnp
import jax.experimental.pallas as pl
import jax.experimental.pallas.tpu as pltpu

F32 = jnp.float32


def _mo(x, m):
    return x if isinstance(x, int) else pl.multiple_of(x, m)


BF16 = jnp.bfloat16

L = 2048
D = 512
N = 128
FF = 1376
T = 128
NB = L // T
NH = 42
NLO = 16
NG = D // 8
RB = 256
HALO = 8


def _bf16_round(l):
    l = int(l)
    if l < 256:
        return l
    e = l.bit_length() - 8
    q, rem = l >> e, l & ((1 << e) - 1)
    half = 1 << (e - 1)
    if rem > half or (rem == half and (q & 1)):
        q += 1
    return q << e


def _hi_values():
    hi = []
    hi += [j for j in range(8)]
    hi += [128 + j for j in range(8)]
    hi += [256 + 128 * h + 2 * q for h in range(2) for q in range(4)]
    hi += [512 + 128 * h + 4 * q for h in range(4) for q in range(2)]
    hi += [1024 + 128 * h for h in range(8)]
    hi += [2048]
    return hi


@functools.lru_cache(maxsize=1)
def _tables():
    hi = _hi_values()
    pos = {}
    for h, hv in enumerate(hi):
        hb, j = h // 8, h % 8
        for lo in range(NLO):
            r = hv + 8 * lo
            lane = 8 * lo + j
            pos.setdefault(r, hb * 128 + lane)
    theta = np.pi * (2 * np.arange(T) + 1) / (2 * T)
    jj = np.arange(T)
    Fm = np.concatenate([np.cos(theta[:, None] * jj[None]), -np.sin(theta[:, None] * jj[None])], 0)
    mm = T + np.arange(T)
    Gm = np.concatenate([np.cos(mm[:, None] * theta[None]), -np.sin(mm[:, None] * theta[None])], 1) / T
    blocks, spans = [], []
    off = 0
    for b in range(NB):
        lags = [l for l in range((b - 1) * T + 1, (b + 1) * T) if 0 <= l < L]
        ps = [pos[_bf16_round(l)] for l in lags]
        t0, t1 = min(ps) // 128, max(ps) // 128
        nt = t1 - t0 + 1
        tab = np.zeros((2 * T, nt * 128), np.float64)
        for l, p in zip(lags, ps):
            m = l - (b - 1) * T
            tab[:T, p - t0 * 128] += np.cos(theta * m)
            tab[T:, p - t0 * 128] += -np.sin(theta * m)
        blocks.append(np.pad(tab, ((0, 0), (0, 256 - nt * 128))))
        if spans and spans[-1][2:] == (t0, nt):
            spans[-1] = (spans[-1][0], b + 1, t0, nt)
        else:
            spans.append((b, b + 1, t0, nt))
    Fx = np.concatenate(blocks, 0)
    return (Fm.astype(np.float32), Gm.astype(np.float32), Fx.astype(np.float32), tuple(spans))


def _cmul(ar, ai, br, bi):
    return ar * br - ai * bi, ar * bi + ai * br


def _sincos(x):
    kf = jnp.floor(x * 0.6366197723675814 + 0.5)
    r = x - kf * 1.5703125
    r = r - kf * 4.837512969970703125e-4
    r = r - kf * 7.54978995489188216e-8
    r2 = r * r
    s = r + r * r2 * (-1.6666654611e-1 + r2 * (8.3321608736e-3 + r2 * (-1.9515295891e-4)))
    c = 1.0 - 0.5 * r2 + r2 * r2 * (4.166664568298827e-2 + r2 * (-1.388731625493765e-3 + r2 * 2.443315711809948e-5))
    q = kf.astype(jnp.int32)
    swap = (q & 1) == 1
    sn = jnp.where(swap, c, s)
    cs = jnp.where(swap, s, c)
    sn = jnp.where((q & 2) == 2, -sn, sn)
    cs = jnp.where(((q + 1) & 2) == 2, -cs, cs)
    return sn, cs


def _ln(x):
    m = jnp.mean(x, axis=-1, keepdims=True)
    xc = x - m
    v = jnp.mean(xc * xc, axis=-1, keepdims=True)
    return xc * jax.lax.rsqrt(v + 1e-5)


def _gelu(x):
    c1 = 0.7978845608028654
    u = x * (x * x * (c1 * 0.044715) + c1)
    hx = 0.5 * x
    return hx + hx * jnp.tanh(u)


def _make_kernel(spans, fx_cols):
    def kernel(are_ref, aim_ref, bre_ref, bim_ref, cre_ref, cim_ref, ldt_ref, dsk_ref,
               fm_ref, gm_ref,
               x_hbm, w1_hbm, w2_hbm, w3_hbm, w4_hbm, fx_hbm,
               out_hbm,
               x_v, w1_v, w2_v, w3_v, w4_v, fx_v, out_v,
               ehi_v, elo_v, kd_v, kdt_v, kh_v, uh_v, yh_v, xn_v, h_v,
               ldt_v, acc_v, x1n_v, kd2_v, in_sems, out_sems):
        def xcopy(k):
            r = pl.ds(_mo(k * RB, RB), RB)
            return pltpu.make_async_copy(x_hbm.at[r, :], x_v.at[r, :], in_sems.at[5 + k])

        copies = [
            pltpu.make_async_copy(fx_hbm, fx_v, in_sems.at[0]),
            pltpu.make_async_copy(w1_hbm, w1_v, in_sems.at[1]),
            pltpu.make_async_copy(w2_hbm, w2_v, in_sems.at[2]),
            pltpu.make_async_copy(w3_hbm, w3_v, in_sems.at[3]),
            pltpu.make_async_copy(w4_hbm, w4_v, in_sems.at[4]),
        ]
        xcopy(0).start()
        copies[1].start()
        for k in range(1, L // RB):
            xcopy(k).start()
        for c in (0, 2, 3, 4):
            copies[c].start()

        ld_row = ldt_ref[...].astype(F32).reshape(1, D)
        ldt_v[...] = jnp.broadcast_to(ld_row, (N, D)).T.astype(BF16)

        CB = 64

        def egen(cb, carry):
            r0 = _mo(cb * CB, CB)
            rows = pl.ds(r0, CB)
            ldt_b = ldt_v[rows, :]
            are_b, aim_b = are_ref[rows, :], aim_ref[rows, :]

            def dtof(l):
                return jnp.exp(l.astype(F32)).astype(BF16).astype(F32)

            def zpow(ar_, ai_, k):
                mag = jnp.exp(ar_ * k)
                sn, cs = _sincos(ai_ * k)
                return mag * cs, mag * sn

            dt_a = dtof(ldt_b)
            for gg in range(CB // 8):
                g = cb * (CB // 8) + gg
                sl = slice(8 * gg, 8 * gg + 8)
                rg = pl.ds(_mo(r0 + 8 * gg, 8), 8)
                dt = dt_a[sl]
                ar = dt * are_b[sl].astype(F32)
                ai = dt * aim_b[sl].astype(F32)
                br = dt * bre_ref[rg, :].astype(F32)
                bi = dt * bim_ref[rg, :].astype(F32)
                cr, ci = _cmul(cre_ref[rg, :].astype(F32), cim_ref[rg, :].astype(F32), br, bi)
                z1 = zpow(ar, ai, 1.0)
                pw = [None, z1]
                for j in range(2, 8):
                    pw.append(_cmul(*pw[-1], *z1))
                w = (pw[4][0] * pw[4][0] - pw[4][1] * pw[4][1], 2.0 * pw[4][0] * pw[4][1])
                v = w
                for _ in range(4):
                    v = (v[0] * v[0] - v[1] * v[1], 2.0 * v[0] * v[1])
                pend = []

                def pack2(ref, idx, v0, v1):
                    for p, ls in ((0, slice(0, N)), (1, slice(N, 2 * N))):
                        ref[g, idx, :, ls] = jnp.concatenate([v0[p], v1[p]], axis=0).astype(BF16)

                def put_hi(h, val):
                    pend.append(val)
                    if h % 2 == 1:
                        pack2(ehi_v, h // 2, pend[0], pend[1])
                        pend.clear()

                cv = (cr, ci)
                for hp in range(17):
                    if hp < 2:
                        js, h0 = list(range(8)), 8 * hp
                    elif hp < 4:
                        js, h0 = [0, 2, 4, 6], 16 + 4 * (hp - 2)
                    elif hp < 8:
                        js, h0 = [0, 4], 24 + 2 * (hp - 4)
                    else:
                        js, h0 = [0], 32 + (hp - 8)
                    for q, j in enumerate(js):
                        put_hi(h0 + q, cv if j == 0 else _cmul(*cv, *pw[j]))
                    if hp < 16:
                        cv = _cmul(*cv, *v)
                zero = jnp.zeros((8, N), F32)
                put_hi(NH - 1, (zero, zero))

                wp = (jnp.ones((8, N), F32), zero)
                prevv = None
                for lo in range(NLO):
                    cur = (wp[0], -wp[1])
                    if lo % 2 == 1:
                        pack2(elo_v, lo // 2, prevv, cur)
                    prevv = cur
                    if lo == 0:
                        wp = w
                    elif lo < NLO - 1:
                        wp = _cmul(*wp, *w)
            return carry

        lane8 = jax.lax.broadcasted_iota(jnp.int32, (8, 128), 1) % 8

        KG = 8

        def kgen(gi, carry):
            for gg in range(KG):
                g = gi * KG + gg
                lhs = ehi_v[g].reshape(NH * 8, 2 * N)
                rhs = elo_v[g].reshape(NLO * 8, 2 * N)
                o = jax.lax.dot_general(lhs, rhs, (((1,), (1,)), ((), ())), preferred_element_type=F32)
                r0 = _mo(g * 8, 8)
                for hb in range(6):
                    acc = jnp.zeros((8, 128), F32)
                    for j in range(8):
                        h = 8 * hb + j
                        if h >= NH - 1:
                            continue
                        blk = pltpu.roll(o[8 * h:8 * h + 8, :], j, 1, stride=7, stride_axis=0)
                        acc = jnp.where(lane8 == j, blk, acc)
                    kd_v[pl.ds(r0, 8), hb * 128:(hb + 1) * 128] = acc
            return carry


        h_v[0:HALO, :] = jnp.zeros((HALO, D), F32)
        for p in range(3):
            uh_v[NB, p] = jnp.zeros((T, D), F32)
        h_v[HALO + L:HALO + L + HALO, :] = jnp.zeros((HALO, D), F32)

        def p1a(k, carry):
            r0 = _mo(k * RB, RB)
            xn = _ln(x_v[pl.ds(r0, RB), :].astype(F32)).astype(BF16)
            xn_v[pl.ds(r0, RB), :] = xn
            xn2 = _ln(xn.astype(F32)).astype(BF16)
            h = _gelu(jnp.dot(xn2, w1_v[...], preferred_element_type=F32))
            h_v[pl.ds(_mo(r0 + HALO, 8), RB), :] = h
            for c in range(RB // T):
                uu = jnp.dot(fm_ref[...], xn[c * T:(c + 1) * T, :], preferred_element_type=F32)
                ci = k * (RB // T) + c
                uh_v[ci, 0] = uu[:T] + uu[T:]
                uh_v[ci, 1] = uu[:T]
                uh_v[ci, 2] = uu[T:]
            return carry

        egen(0, 0)
        egen(1, 0)
        kgen(0, 0)
        copies[1].wait()

        def merged(k, carry):
            xcopy(k - 1).wait()
            egen(k + 1, 0)
            kgen(k, 0)
            p1a(k - 1, 0)
            return carry

        jax.lax.fori_loop(1, L // RB - 1, merged, 0)
        xcopy(L // RB - 2).wait()
        xcopy(L // RB - 1).wait()
        kgen(L // RB - 1, 0)
        p1a(L // RB - 2, 0)
        p1a(L // RB - 1, 0)
        lane8w = jax.lax.broadcasted_iota(jnp.int32, (8, D), 1) % 8
        for tl in range(6):
            kt = kd_v[:, tl * 128:(tl + 1) * 128].T
            for i in range(16):
                o_ = kt[8 * i:8 * i + 8, :]
                for r in range(1, 8):
                    i2 = (i + r) % 16
                    o_ = jnp.where(lane8w == r, kt[8 * i2:8 * i2 + 8, :], o_)
                kd2_v[tl * 128 + 8 * i:tl * 128 + 8 * i + 8, :] = o_
        kdt_v[...] = kd2_v[...].astype(BF16)

        copies[0].wait()
        for (b0, b1, t0, nt) in spans:
            kk = jnp.dot(fx_v[b0 * 2 * T:b1 * 2 * T, 0:nt * 128], kdt_v[t0 * 128:(t0 + nt) * 128, :],
                         preferred_element_type=F32)
            for b in range(b0, b1):
                o_ = (b - b0) * 2 * T
                kc, kd_ = kk[o_:o_ + T], kk[o_ + T:o_ + 2 * T]
                kh_v[b, 0] = kc
                kh_v[b, 1] = kd_ - kc
                kh_v[b, 2] = kc + kd_


        copies[2].wait()
        copies[3].wait()
        copies[4].wait()
        C4 = D // 4
        R = 8

        LH = 256

        MH = 4

        def p1b(mm, carry):
            cis = []
            for hf in range(MH):
                cis += [MH * mm + hf, NB // 2 - 1 - (MH * mm + hf)]
            rows = [_mo(ci * RB, RB) for ci in cis]

            def pointwise(sbi):
                hf = sbi // 32
                sbi = sbi % 32
                m = MH * mm + hf
                split = 2 * m + 2
                if isinstance(sbi, int):
                    sb, l0 = (sbi // 2) * R, (sbi % 2) * LH
                else:
                    sb, l0 = _mo((sbi // 2) * R, R), _mo((sbi % 2) * LH, LH)
                rs = pl.ds(sb, R)
                rs2 = pl.ds(_mo(sb + T, R), R)
                ls = pl.ds(l0, LH)

                def ldu(i):
                    return [uh_v[i, p, rs, ls] for p in range(3)]

                accA = accB = snap = None
                ucur = None
                for s in range(NB + 2):
                    if s < 2:
                        b, top = s, 2 * m + 1
                    elif s >= 8:
                        b, top = s - split, NB - 1 - 2 * m
                    else:
                        first = s < split
                        b = jnp.where(first, s, s - split)
                        top = jnp.where(first, 2 * m + 1, NB - 1 - 2 * m)
                    if s in (2, 4, 6, 8):
                        if snap is None:
                            snap = accA + accB
                        else:
                            at = split == s
                            snap = [jnp.where(at, x_, y_) for x_, y_ in zip(accA + accB, snap)]
                    if s in (0, 2, 4, 6, 8):
                        ucur = ldu(top - b)
                    kk = [kh_v[b, p, rs, ls] for p in range(3)]
                    pa = [k_ * u_ for k_, u_ in zip(kk, ucur)]
                    accA = pa if accA is None else [x_ + y_ for x_, y_ in zip(accA, pa)]
                    if s == NB + 1:
                        break
                    nxt = top - b - 1
                    if s <= 7:
                        nxt = jnp.where(nxt < 0, NB, nxt)
                    unext = ldu(nxt)
                    pb = [k_ * u_ for k_, u_ in zip(kk, unext)]
                    accB = pb if accB is None else [x_ + y_ for x_, y_ in zip(accB, pb)]
                    ucur = unext
                tot = accA + accB
                sec = [x_ - y_ for x_, y_ in zip(tot, snap)]
                for c, ss in ((1, snap[0:3]), (0, snap[3:6]), (3, sec[0:3]), (2, sec[3:6])):
                    yh_v[4 * hf + c, rs, ls] = ss[0] - ss[2]
                    yh_v[4 * hf + c, rs2, ls] = ss[0] + ss[1]

            xns, hss = [], []
            for c in range(2 * MH):
                xns.append(xn_v[pl.ds(rows[c], RB), :])
                win = h_v[pl.ds(rows[c], RB + 2 * HALO), :]
                hss.append(jnp.concatenate([
                    win[HALO - 1:HALO - 1 + RB, 0 * C4:1 * C4],
                    win[HALO + 1:HALO + 1 + RB, 1 * C4:2 * C4],
                    win[HALO - 2:HALO - 2 + RB, 2 * C4:3 * C4],
                    win[HALO + 2:HALO + 2 + RB, 3 * C4:4 * C4]], axis=-1).astype(BF16))
            hs = jnp.concatenate(hss, 0)
            x1 = jnp.concatenate(xns, 0).astype(F32) + jnp.dot(hs, w2_v[...], preferred_element_type=F32)
            acc_v[...] = x1
            x1n_v[...] = _ln(x1).astype(BF16)
            FC, PRE, INN = 384, 5, 41
            for q in range(PRE):
                pointwise(q)

            def ffchunk(w3c, w4c):
                h3 = _gelu(jax.lax.dot_general(x1n_v[...], w3c, (((1,), (1,)), ((), ())),
                                               preferred_element_type=F32))
                acc_v[...] += jnp.dot(h3.astype(BF16), w4c, preferred_element_type=F32)

            def inner(c, carry2):
                c0 = _mo(c * FC, 16)
                ffchunk(w3_v[pl.ds(c0, FC), :], w4_v[pl.ds(c0, FC), :])
                for q in range(INN):
                    pointwise(PRE + INN * c + q)
                return carry2

            NFC = FF // FC
            jax.lax.fori_loop(0, NFC, inner, 0)
            if NFC * FC < FF:
                ffchunk(w3_v[NFC * FC:FF, :], w4_v[NFC * FC:FF, :])
            for q in range(PRE + INN * NFC, MH * 2 * T // R):
                pointwise(q)
            for c in range(2 * MH):
                ys = [jnp.dot(gm_ref[...], yh_v[2 * c + q].astype(BF16), preferred_element_type=F32)
                      for q in range(2)]
                y = jnp.concatenate(ys, 0).astype(BF16)
                bb = acc_v[c * RB:(c + 1) * RB, :]
                xnf = xn_v[pl.ds(rows[c], RB), :].astype(F32)
                s = y.astype(F32) + xnf * dsk_ref[...].astype(F32).reshape(1, D)
                o = x_v[pl.ds(rows[c], RB), :].astype(F32) + s * (bb * jax.nn.sigmoid(bb))
                out_v[pl.ds(rows[c], RB), :] = o.astype(BF16)
                ci = cis[c]
                pltpu.make_async_copy(out_v.at[pl.ds(rows[c], RB), :], out_hbm.at[pl.ds(rows[c], RB), :],
                                      out_sems.at[ci]).start()
            return carry

        jax.lax.fori_loop(0, NB // 4 // MH, p1b, 0)

        for ci in range(NB // 2):
            pltpu.make_async_copy(out_v.at[pl.ds(ci * RB, RB), :], out_hbm.at[pl.ds(ci * RB, RB), :],
                                  out_sems.at[ci]).wait()

    return kernel


@jax.jit
def pallas_recurrent_scan__ssm_conv_s4__mixer_s_mlp__prompt_kernel(
    A_u: jax.Array,
    A_A_re: jax.Array,
    A_A_im: jax.Array,
    A_B_re: jax.Array,
    A_B_im: jax.Array,
    A_C_re: jax.Array,
    A_C_im: jax.Array,
    A_log_dt: jax.Array,
    A_Dskip: jax.Array,
    B_x: jax.Array,
    B_w1: jax.Array,
    B_w2: jax.Array,
    B_w3: jax.Array,
    B_w4: jax.Array,
):
    Fm, Gm, Fx, spans = _tables()
    fx_cols = Fx.shape[1]
    x = A_u.reshape(L, D)

    vm = pl.BlockSpec(memory_space=pltpu.VMEM)
    hbm = pl.BlockSpec(memory_space=pl.ANY)
    out = pl.pallas_call(
        _make_kernel(spans, fx_cols),
        out_shape=jax.ShapeDtypeStruct((L, D), BF16),
        in_specs=[vm] * 10 + [hbm] * 6,
        out_specs=hbm,
        scratch_shapes=[
            pltpu.VMEM((L, D), BF16),
            pltpu.VMEM((D, D), BF16),
            pltpu.VMEM((D, D), BF16),
            pltpu.VMEM((FF, D), BF16),
            pltpu.VMEM((FF, D), BF16),
            pltpu.VMEM((NB * 2 * T, fx_cols), BF16),
            pltpu.VMEM((L, D), BF16),
            pltpu.VMEM((NG, NH // 2, 16, 2 * N), BF16),
            pltpu.VMEM((NG, NLO // 2, 16, 2 * N), BF16),
            pltpu.VMEM((D, 6 * 128), F32),
            pltpu.VMEM((6 * 128, D), BF16),
            pltpu.VMEM((NB, 3, T, D), F32),
            pltpu.VMEM((NB + 1, 3, T, D), F32),
            pltpu.VMEM((16, 2 * T, D), F32),
            pltpu.VMEM((L, D), BF16),
            pltpu.VMEM((L + 2 * HALO, D), F32),
            pltpu.VMEM((D, N), BF16),
            pltpu.VMEM((8 * RB, D), F32),
            pltpu.VMEM((8 * RB, D), BF16),
            pltpu.VMEM((6 * 128, D), F32),
            pltpu.SemaphoreType.DMA((5 + L // RB,)),
            pltpu.SemaphoreType.DMA((NB // 2,)),
        ],
        compiler_params=pltpu.CompilerParams(vmem_limit_bytes=100 * 1024 * 1024),
    )(A_A_re, A_A_im, A_B_re, A_B_im, A_C_re, A_C_im, A_log_dt, A_Dskip,
      jnp.asarray(Fm, BF16), jnp.asarray(Gm, BF16),
      x, B_w1, B_w2, B_w3.T, B_w4, jnp.asarray(Fx, BF16))
    return out.reshape(1, L, D)
```
